```python
import os as _os
_os.environ.setdefault("JAX_PLATFORMS", "cpu")
import jax
import jax.numpy as jnp

def _softmax(x, axis=-1):
    return jax.nn.softmax(x, axis=axis)
def _gelu(x):
    return jax.nn.gelu(x, approximate=True)
def _silu(x):
    return jax.nn.silu(x)
def _sigmoid(x):
    return jax.nn.sigmoid(x)
def _layernorm(x, axis=-1, eps=1e-5):
    m = jnp.mean(x, axis=axis, keepdims=True)
    v = jnp.var(x, axis=axis, keepdims=True)
    return (x - m) / jnp.sqrt(v + eps)
def _scatter_add(tgt, idx, src, axis=0):
    return tgt.at[idx].add(src)
def _segment_sum(src, seg, n):
    return jax.ops.segment_sum(src, seg, n)
class _Rng:
    def __init__(self, key):
        self._k = key
    def _next(self):
        self._k, sub = jax.random.split(self._k)
        return sub
    def normal(self, shape):
        return jax.random.normal(self._next(), shape, dtype=jnp.bfloat16)
    def randint(self, lo, hi, shape):
        return jax.random.randint(self._next(), shape, lo, hi, dtype=jnp.int32)
    def uniform(self, shape, lo=0.0, hi=1.0):
        return jax.random.uniform(self._next(), shape, jnp.bfloat16, lo, hi)
    def permutation(self, n):
        return jax.random.permutation(self._next(), n)


kernel_name = 'sequential_preLN__softmax_full_mha__dense_activation_squared_relu__prompt'

def setup_inputs():
    _rng = _Rng(jax.random.key(int.from_bytes(__import__("os").urandom(4), "little")))
    _w = (lambda a: (lambda t: t.astype(jnp.bfloat16) if jnp.issubdtype(t.dtype, jnp.floating) else t)(jnp.asarray(a)))
    def _A_setup():
        B, S, D = 1, 2048, 448
        return {
            "x": _w((lambda *s: _rng.normal(s) * 0.05)(B, S, D)),
            "wqkv": _w((lambda *s: _rng.normal(s) * 0.05)(D, 3 * D)),
            "wo": _w((lambda *s: _rng.normal(s) * 0.05)(D, D)),
        }
    _A_in = _A_setup()

    def _B_setup():
        B, S, D, F = 1, 2048, 448, 1792
        return {
            "x": _w((lambda *s: _rng.normal(s) * 0.05)(B, S, D)),
            "w1": _w((lambda *s: _rng.normal(s) * 0.05)(D, F)),
            "b1": _w((lambda *s: _rng.normal(s) * 0.05)(F)),
            "w2": _w((lambda *s: _rng.normal(s) * 0.05)(F, D)),
            "b2": _w((lambda *s: _rng.normal(s) * 0.05)(D)),
        }
    _B_in = _B_setup()

    return {
        "A_x": _A_in["x"],
        "A_wqkv": _A_in["wqkv"],
        "A_wo": _A_in["wo"],
        "B_x": _B_in["x"],
        "B_w1": _B_in["w1"],
        "B_b1": _B_in["b1"],
        "B_w2": _B_in["w2"],
        "B_b2": _B_in["b2"],
    }

def reference(A_x, A_wqkv, A_wo, B_x, B_w1, B_b1, B_w2, B_b2):
    def _A_ref(x, wqkv, wo):
        B, S, D = x.shape
        H = 16; Dh = D // H
        qkv = (lambda x, *d: x.transpose(*d))((x @ wqkv).reshape(B, S, 3, H, Dh), 2, 0, 3, 1, 4)
        q, k, v = qkv[0], qkv[1], qkv[2]
        scale = Dh ** -0.5
        scores = jnp.einsum("bhqd,bhkd->bhqk", q, k) * scale
        p = _softmax(scores, axis=-1)
        o = jnp.einsum("bhqk,bhkd->bhqd", p, v)
        return (lambda x, *d: x.transpose(*d))(o, 0, 2, 1, 3).reshape(B, S, D) @ wo

    def _B_ref(x, w1, b1, w2, b2):
        h = jnp.einsum("bsd,df->bsf", x, w1) + b1
        zero = jnp.zeros_like(h)
        r = jnp.where(h > zero, h, zero)
        h = r * r
        out = jnp.einsum("bsf,fd->bsd", h, w2) + b2
        return out

    x = A_x
    h = x + _A_ref(_layernorm(x, axis=-1), A_wqkv, A_wo)
    h2 = h + _B_ref(_layernorm(h, axis=-1), B_w1, B_b1, B_w2, B_b2)
    return h2
```

```python
import functools
import math

import jax
import jax.numpy as jnp
from jax import lax
import jax.experimental.pallas as pl
import jax.experimental.pallas.tpu as pltpu

S, D, H, F = 2048, 448, 16, 1792
DH = D // H
TB = 512
NB = S // TB
KT = 128
GH = 4
GR = GH * DH
EPS = 1e-5
QSCALE = DH ** -0.5 * math.log2(math.e)
F32, BF16 = jnp.float32, jnp.bfloat16


def _ln_t(x):
    m = jnp.sum(x, axis=0, keepdims=True) * (1.0 / D)
    c = x - m
    v = jnp.sum(c * c, axis=0, keepdims=True) * (1.0 / D)
    return c * lax.rsqrt(v + EPS)


def _dot(a, b):
    return jnp.dot(a, b, preferred_element_type=F32)


def _kernel(x_hbm, wqkv_hbm, wo_hbm, w1_hbm, b1_ref, w2t_hbm, b2_ref, out_hbm,
            x_v, wqkv_v, wo_v, w1_v, w2t_v, wqkvt, wot, w1t, b2c,
            q_s, k_s, v_s, s_s, m_s, o_s, a_s, out_v, in_sem, out_sem, *, cfg):
    x_cp = [pltpu.make_async_copy(x_hbm.at[:, b * TB:(b + 1) * TB], x_v.at[b], in_sem.at[b])
            for b in range(NB)]
    wqkv_cp = pltpu.make_async_copy(wqkv_hbm, wqkv_v, in_sem.at[NB])
    wo_cp = pltpu.make_async_copy(wo_hbm, wo_v, in_sem.at[NB + 1])
    w1_cp = pltpu.make_async_copy(w1_hbm, w1_v, in_sem.at[NB + 2])
    w2_cp = pltpu.make_async_copy(w2t_hbm, w2t_v, in_sem.at[NB + 3])
    wqkv_cp.start()
    for c in x_cp:
        c.start()
    wo_cp.start()
    w1_cp.start()
    w2_cp.start()

    wqkv_cp.wait()
    wqkvt[...] = wqkv_v[...].T
    for c in x_cp:
        c.wait()

    sub = lax.broadcasted_iota(jnp.int32, (8, TB), 0)
    MA = cfg.get("MA", 112)

    def proj(b, carry):
        xn = _ln_t(x_v[b].astype(F32)).astype(BF16)
        zpad = jnp.zeros((128 - GR, TB), BF16)
        for g in range(H // GH):
            q = _dot(wqkvt[g * GR:(g + 1) * GR, :], xn)
            q_s[b, g] = jnp.concatenate([(q * QSCALE).astype(BF16), zpad], axis=0)
        for g in range(H // GH):
            k = _dot(wqkvt[D + g * GR:D + (g + 1) * GR, :], xn)
            k_s[g, b] = jnp.concatenate([k.astype(BF16), zpad], axis=0).T
        for g in range(H // GH):
            v = _dot(wqkvt[2 * D + g * GR:2 * D + (g + 1) * GR, :], xn)
            for p in range(2):
                r = 56 * p
                mid = v[r + 24:r + 32]
                ev = jnp.concatenate([v[r:r + 24], jnp.where(sub < 4, mid, 1.0)], axis=0)
                od = jnp.concatenate([jnp.where(sub < 4, 1.0, mid), v[r + 32:r + 56]], axis=0)
                v_s[g * GH + 2 * p, b] = ev.astype(BF16)
                v_s[g * GH + 2 * p + 1, b] = od.astype(BF16)
        return carry

    lax.fori_loop(0, NB, proj, 0)

    def masked_q(h, b):
        g = h // GH
        lo = (h % GH) * (DH // 2)
        w = pltpu.bitcast(q_s[b, g], jnp.uint32)
        row = lax.broadcasted_iota(jnp.int32, w.shape, 0)
        keep = jnp.logical_and(row >= lo, row < lo + DH // 2)
        return pltpu.bitcast(jnp.where(keep, w, jnp.uint32(0)), BF16)

    def attn_stage(h_qk, h_pv):
        for b in range(NB):
            if h_qk is not None:
                q = masked_q(h_qk, b)
                g = h_qk // GH
            if h_pv is not None:
                m = m_s[b]
            acc = None
            mx = None
            for j in range(S // KT):
                kb, ko = divmod(j * KT, TB)
                rows = slice(j * KT, (j + 1) * KT)
                if h_pv is not None:
                    s_old = s_s[b, rows, :].reshape(KT // 8, 8, TB)
                    p = jnp.exp2(s_old - m[None]).reshape(KT, TB).astype(BF16)
                if h_qk is not None:
                    s = _dot(k_s[g, kb, ko:ko + KT, :], q)
                    s_s[b, rows, :] = s
                    t = jnp.max(s.reshape(KT // 8, 8, TB), axis=0)
                    mx = t if mx is None else jnp.maximum(mx, t)
                if h_pv is not None:
                    d = _dot(v_s[h_pv, kb, :, ko:ko + KT], p)
                    acc = d if acc is None else acc + d
            if h_pv is not None:
                o_s[b, h_pv] = acc
            if h_qk is not None:
                m_s[b] = jnp.broadcast_to(jnp.max(mx, axis=0, keepdims=True), (8, TB))

    attn_stage(0, None)

    def head_body(h, carry):
        attn_stage(h + 1, h)
        return carry

    lax.fori_loop(0, H - 1, head_body, 0)

    wo_cp.wait()
    w1_cp.wait()
    w2_cp.wait()
    wot[...] = wo_v[...].T
    b1row = jnp.where(lax.broadcasted_iota(jnp.int32, (64, F), 0) == 0,
                      b1_ref[...].astype(F32), 0.0).astype(BF16)
    w1t[...] = jnp.concatenate([w1_v[...], b1row], axis=0).T
    b2c[...] = jnp.broadcast_to(b2_ref[...].astype(F32), (128, D)).T

    attn_stage(None, H - 1)

    MC = cfg.get("MC", 128)
    MD = cfg.get("MD", 64)

    def out_copy(b):
        return pltpu.make_async_copy(
            out_v.at[b], out_hbm.at[:, pl.ds(pl.multiple_of(b * TB, TB), TB)], out_sem.at[b])

    def ffn(b, carry):
        parts = []
        for p in range(H // 2):
            ev = o_s[b, 2 * p]
            od = o_s[b, 2 * p + 1]
            ev = ev * (1.0 / ev[31:32])
            od = od * (1.0 / od[0:1])
            parts += [ev[:24], jnp.where(sub < 4, ev[24:], od[:8]), od[8:]]
        on = jnp.concatenate(parts, axis=0).astype(BF16)
        h = x_v[b].astype(F32) + jnp.concatenate(
            [_dot(wot[r:r + MD, :], on) for r in range(0, D, MD)], axis=0)
        ones = jnp.ones((64, TB), BF16)
        hn = jnp.concatenate([_ln_t(h).astype(BF16), ones], axis=0)
        for r in range(0, F, MC):
            u = jnp.maximum(_dot(w1t[r:r + MC, :], hn), 0.0)
            a_s[r:r + MC, :] = (u * u).astype(BF16)
        a = a_s[...]
        for r in range(0, D, MD):
            y = _dot(w2t_v[r:r + MD, :], a) + h[r:r + MD] + jnp.tile(b2c[r:r + MD, :], (1, TB // 128))
            out_v[b, r:r + MD, :] = y.astype(BF16)
        out_copy(b).start()
        return carry

    lax.fori_loop(0, NB, ffn, 0)
    for b in range(NB):
        out_copy(b).wait()


def build(cfg):
    def fn(A_x, A_wqkv, A_wo, B_x, B_w1, B_b1, B_w2, B_b2):
        del B_x
        hbm = pl.BlockSpec(memory_space=pltpu.HBM)
        vmem = pl.BlockSpec(memory_space=pltpu.VMEM)
        out_t = pl.pallas_call(
            functools.partial(_kernel, cfg=cfg),
            out_shape=jax.ShapeDtypeStruct((D, S), BF16),
            in_specs=[hbm, hbm, hbm, hbm, vmem, hbm, vmem],
            out_specs=hbm,
            scratch_shapes=[
                pltpu.VMEM((NB, D, TB), BF16),
                pltpu.VMEM((D, 3 * D), BF16),
                pltpu.VMEM((D, D), BF16),
                pltpu.VMEM((D, F), BF16),
                pltpu.VMEM((D, F), BF16),
                pltpu.VMEM((3 * D, D), BF16),
                pltpu.VMEM((D, D), BF16),
                pltpu.VMEM((F, 512), BF16),
                pltpu.VMEM((D, 128), F32),
                pltpu.VMEM((NB, H // GH, 128, TB), BF16),
                pltpu.VMEM((H // GH, NB, TB, 128), BF16),
                pltpu.VMEM((H, NB, 32, TB), BF16),
                pltpu.VMEM((NB, S, TB), F32),
                pltpu.VMEM((NB, 8, TB), F32),
                pltpu.VMEM((NB, H, 32, TB), F32),
                pltpu.VMEM((F, TB), BF16),
                pltpu.VMEM((NB, D, TB), BF16),
                pltpu.SemaphoreType.DMA((NB + 4,)),
                pltpu.SemaphoreType.DMA((NB,)),
            ],
            compiler_params=pltpu.CompilerParams(vmem_limit_bytes=100 * 1024 * 1024),
            name="fused_block",
        )(A_x[0].T, A_wqkv, A_wo, B_w1, B_b1.reshape(1, F), B_w2.T, B_b2.reshape(1, D))
        return out_t.T[None]
    return jax.jit(fn)


pallas_sequential_preLN__softmax_full_mha__dense_activation_squared_relu__prompt_kernel = build({})
```

```python
import functools
import math

import jax
import jax.numpy as jnp
from jax import lax
import jax.experimental.pallas as pl
import jax.experimental.pallas.tpu as pltpu

S, D, H, F = 2048, 448, 16, 1792
DH = D // H
TB = 512
HB = TB // 2
NB = S // TB
NT = TB // 128
KT = 128
NJ = S // KT
GH = 4
GR = GH * DH
NV = 256
PAD = 32
EPS = 1e-5
QSCALE = DH ** -0.5 * math.log2(math.e)
BOUND = 40.0
F32, BF16, U32 = jnp.float32, jnp.bfloat16, jnp.uint32
P = functools.partial


def _pack(x):
    return pltpu.bitcast(x.astype(BF16), U32)


def _unpack(w):
    return pltpu.bitcast(w, BF16)


def _round(x):
    return x.astype(BF16).astype(F32)


def _matmul(a, b):
    return lax.dot_general(a, b, (((1,), (0,)), ((), ())), preferred_element_type=F32)


def _low(x):
    return lax.broadcasted_iota(jnp.int32, x.shape, 0) < 4


def _at(row, n):
    return pl.ds(pl.multiple_of(row, 8), n)


def _run(*streams):
    timed = []
    for k, stream in enumerate(streams):
        jobs, start, stop = stream if isinstance(stream, tuple) else (stream, 0.0, 1.0)
        timed += [(start + (stop - start) * (n + 0.5) / len(jobs), k, n, job) for n, job in enumerate(jobs)]
    for entry in sorted(timed, key=lambda e: e[:3]):
        entry[3]()


def _kernel(x_hbm, wqkv_hbm, wo_hbm, w1_hbm, b1_hbm, w2t_hbm, b2_hbm, out_hbm,
            x_v, wqkv_v, wo_v, w1_v, w2t_v, wq_t, wk_raw, wk_t, wo_raw, wo_t, w1_t, w2_t, b1_c, b2_c,
            xn_s, st_s, q_s, qf_s, sh_s, kt_s, k_s, kf_s, kb_s, v_s, p_s, o_s, ol_s, on_s, h_s, a_s, out_v,
            b1_v, b2_v, z_s, in_sem, out_sem):
    def x_copy(b):
        return x_hbm.at[:, b * TB:(b + 1) * TB], x_v[b].at[0, 0:D]

    def w_copy(lo, hi):
        return wqkv_hbm.at[:, lo:hi], wqkv_v.at[:, lo:hi]

    loads = [[pltpu.make_async_copy(src, dst, in_sem.at[n]) for src, dst in group] for n, group in enumerate((
        (x_copy(0),),
        (w_copy(0, 256), w_copy(896, 1152)),
        (w_copy(256, 512), w_copy(1152, None)),
        (w_copy(512, 896), x_copy(1)),
        (x_copy(2), x_copy(3), (wo_hbm, wo_v), (b1_hbm, b1_v), (b2_hbm, b2_v)),
        ((w1_hbm, w1_v), (w2t_hbm, w2t_v.at[0:D]))))]
    for group in loads:
        for cp in group:
            cp.start()

    def arrive(n):
        for cp in loads[n]:
            cp.wait()

    def set_zero(i, carry):
        z_s[i] = 0
        return carry

    lax.fori_loop(0, 2, set_zero, 0)
    z = z_s[0]
    tiles = [slice(c, c + 128) for c in range(0, TB, 128)]
    recent = []
    streaming = [None]
    lhs_queue = []

    def dot(a, b):
        y = _matmul(a, b)
        recent.extend(y[-8:, c:c + 128] for c in range(0, y.shape[1], 128))
        return y

    def window(jobs, src, dst, pin, back=16):
        out = [None]

        def step(n):
            if n > 0:
                ref = streaming[0] if pin is None else pin
                w = dst[0][0, _at(32 * z + dst[1], 8), 0:128] if out[0] is None else out[0]
                ref[0, _at(64 * z, 8), 0:w.shape[1]] = w if w.dtype == ref.dtype else pltpu.bitcast(w, ref.dtype)
            if n < len(jobs):
                if len(recent) >= back:
                    w = recent[-back] if src.dtype == F32 else pltpu.bitcast(recent[-back], src.dtype)
                    src[pl.ds(0, w.shape[0]), 0:128] = w
                out[0] = jobs[n]()
        return [P(step, n) for n in range(len(jobs) + 1)]

    def spare(ref):
        return ref.at[5 * z, pl.ds(D, 16)]

    def rounds(passes):
        def job(group, got, i):
            streaming[0] = group[-1][0]
            for (w, r0, _, c, _), rows in zip(group, got):
                rows.append(w.at[z][pl.ds(PAD + r0 // 2 + 8 * i, 8), c * 128:(c + 1) * 128])
            if 16 * (i + 1) == group[0][2]:
                for entry, rows in zip(group, got):
                    lhs_queue.append(_unpack(jnp.concatenate(rows, axis=0)))
                    next(entry[4])
        jobs = []
        for k in range(0, len(passes), 4):
            got = [[] for _ in range(4)]
            jobs += [P(job, passes[k:k + 4], got, i) for i in range(passes[k][2] // 16)]
        return jobs

    def ln_add(acc, st, c, x):
        if not acc:
            acc.update(c=x[0:1], n=0)
        d = x - acc["c"]
        for key, v in (("s1", d), ("s2", d * d)):
            v = jnp.sum(v.reshape(-1, 8, x.shape[1]), axis=0)
            acc[key] = v if acc["n"] == 0 else acc[key] + v
        acc["n"] += x.shape[0]
        if acc["n"] == D:
            m = jnp.sum(acc["s1"], axis=0, keepdims=True) * (1.0 / D)
            var = jnp.sum(acc["s2"], axis=0, keepdims=True) * (1.0 / D) - m * m
            st[0, 0:8, c] = jnp.broadcast_to(m + acc["c"], acc["s1"].shape)
            st[0, 8:16, c] = jnp.broadcast_to(lax.rsqrt(jnp.maximum(var, 0.0) + EPS), acc["s1"].shape)
        return acc["s2"]

    def ln_stats(src, st):
        def job(acc, c, r):
            return ln_add(acc, st, c, src.at[z][r:r + 32, c].astype(F32))
        return [P(job, acc, c, r) for acc, c in (({}, slice(0, HB)), ({}, slice(HB, TB))) for r in range(0, D, 32)]

    def ln_operands(src, st, dst):
        def rows(e, r0, n):
            c = slice(e * HB, (e + 1) * HB)
            x = src.at[3 * z][r0:r0 + n, c].astype(F32).reshape(n // 8, 8, HB)
            return ((x - st[z, 0:8, c][None]) * st[z, 8:16, c][None]).reshape(n, HB)

        def put(t, r, val):
            dst.at[0][pl.ds(64 * t + r // 2, val.shape[0] // 2), :] = _pack(val)

        def mixed(r):
            (x1, x2), (y1, y2) = ([rows(e, o + r, 16) for o in (0, 128)] for e in range(2))
            for t, v in zip((0, 1, 2, 4, 5, 6, 7), (y2, y1 - y2, x2 + y2, x1 + y2, x2 - x1, x1, x1 + y1)):
                put(t, r, v)

        def own(e):
            put((3, 8)[e], 0, rows(e, 256, 64))

        def shared(r):
            e = (r - 320) // 64
            other = _round(rows(1 - e, r, 32))
            put(9, r - 320, other)
            put((3, 8)[e], 64 + r % 64, rows(e, r, 32) - other)

        return ([P(mixed, r) for r in range(0, 128, 16)] + [P(own, 0), P(own, 1)]
                + [P(shared, r) for r in range(320, D, 32)])

    def w_tiles(src, c):
        return (src[320:448, c], src[0:128, c], src[128:256, c], src[256:384, c],
                jnp.concatenate([src[256:320, c], src[384:448, c]], axis=0))

    def w_mix(wa, wb):
        (ta, a11, a12, ua, va), (tb, a21, a22, ub, vb) = wa, wb
        f11, f12, f21, f22 = (w.astype(F32) for w in (a11, a12, a21, a22))
        return (ta, va, f11 + f12, a11, f12 - f22, ua, f11 + f22, a22, f21 + f22, tb, ub, f21 - f11, vb)

    def prep_quad(src, ca, cb, n, dsts):
        for t, w in enumerate(w_mix(w_tiles(src, slice(ca, ca + n)), w_tiles(src, slice(cb, cb + n)))):
            w = pltpu.bitcast(w.astype(BF16).T, U32)
            for dst, r0, lo, hi in dsts:
                dst.at[0][pl.ds(PAD + r0 // 2, (hi - lo) // 2), t * 128:(t + 1) * 128] = w[lo // 2:hi // 2]

    def prep_raw(src, dst, c0, n, r0):
        for t, w in enumerate(w_tiles(src, slice(c0, c0 + n))):
            dst.at[0][pl.ds(PAD + r0 // 2, n // 2), t * 128:(t + 1) * 128] = pltpu.bitcast(w.T, U32)

    def mix_raw(mix, raw, dst, first, pin):
        def job(r):
            wa, wb = ([_unpack(raw.at[z][pl.ds(PAD + (first + r // GR * GR + r + o) // 2, 8), c:c + 128])
                       for c in range(0, 640, 128)] for o in (0, GR))
            for t, w in enumerate(mix(wa, wb)):
                dst.at[0][pl.ds(PAD + r // 2, 8), t * 128:(t + 1) * 128] = _pack(w)
        return window([P(job, r) for r in range(0, 2 * GR, 16)], raw.at[5 * z], (dst, PAD), pin, 8)

    def quad(w, src, r0, n, cols, done, bias=None):
        gen = mm_quad(src, r0, n, cols, done, bias)
        return [(w, r0, n, c, gen) for c in range(13)]

    def mm_quad(src, r0, n, cols, done, bias):
        def mm(t):
            return dot(lhs_queue.pop(), _unpack(src.at[z][pl.ds(64 * t, 64), cols]))

        ta = mm(9)
        if bias is not None:
            ta = ta + bias[z, pl.ds(r0 + PAD, n), :]
        yield
        ay = mm(8) + ta
        yield
        m5 = mm(0)
        ax, ay = ta - m5, ay + m5
        yield
        m3 = mm(1)
        done(0, 1, ay + m3)
        yield
        ax = mm(2) + ax
        yield
        ax = mm(3) + ax
        yield
        m1 = mm(4)
        ax, by = ax + m1, m3 + m1
        yield
        m4 = mm(5)
        done(0, 0, ax + m4)
        yield
        m2 = mm(6)
        bx, by = m4 + m2, by - m2
        yield
        tb = mm(9)
        if bias is not None:
            tb = tb + bias[z, pl.ds(F // 2 + r0 + PAD, n), :]
        bx, by = bx + tb, by + tb
        yield
        done(1, 0, mm(3) + bx)
        yield
        by = mm(7) + by
        yield
        done(1, 1, mm(8) + by)
        yield

    unsafe = [jnp.zeros((8, 128), F32)]

    def split_pair(y, p, fill):
        r = 2 * DH * p
        mid = y[r + 24:r + 32]
        return (jnp.concatenate([y[r:r + 24], jnp.where(_low(mid), mid, fill)], axis=0),
                jnp.concatenate([jnp.where(_low(mid), fill, mid), y[r + 32:r + 56]], axis=0))

    def checked_norm(w, scale):
        n2 = jnp.broadcast_to(jnp.sum(w * w, axis=0, keepdims=True), (8, 128)) * scale
        unsafe[0] = jnp.where(n2 <= BOUND, unsafe[0], 1.0)
        return n2

    def put_q(g, b, t, q):
        q = q * QSCALE
        for p in range(2):
            for e, w in enumerate(split_pair(q, p, 0.0)):
                h = g * GH + 2 * p + e
                shift = _round((checked_norm(w, 1.0 / QSCALE) + BOUND) * -0.5)
                qf_s[b][0, h, :, tiles[t]] = w
                sh_s[b][0, h, :, tiles[t]] = shift
                q_s[b].at[0][pl.ds(h * 16, 16), tiles[t]] = _pack(split_pair(q, p, 0.25 * shift)[e])

    def put_k(g, b, t, k):
        for p in range(2):
            for e, w in enumerate(split_pair(k, p, 0.0)):
                h = g * GH + 2 * p + e
                checked_norm(w, QSCALE)
                kt_s[b].at[0][pl.ds(h * 16, 16), tiles[t]] = _pack(split_pair(k, p, 1.0)[e])
                if b * TB + t * 128 < NV:
                    kf_s[0, h, t] = w

    def put_v(g, b, t, v):
        for p in range(2):
            for e, w in enumerate(split_pair(v, p, 1.0)):
                v_s.at[0][pl.ds(PAD + ((g * GH + 2 * p + e) * NB + b) * 16, 16), tiles[t]] = _pack(w)

    def keys_to_rows(h, b):
        lo = 128 if b == 0 else 0
        k = pltpu.bitcast(_unpack(kt_s[b].at[z][pl.ds(h * 16, 16), lo:]).T, U32)
        k_s.at[0][pl.ds(PAD + (h * S + b * TB + lo) // 2, (TB - lo) // 2), 0:32] = k

    def prep_qv(c):
        n = min(128, D - c)
        prep_quad(wqkv_v, c, 2 * D + c, n,
                  [(wq_t[g], max(c - g * GR, 0), max(g * GR - c, 0), min((g + 1) * GR - c, n))
                   for g in range(c // GR, (c + n - 1) // GR + 1)])

    def project(b, items):
        def done(sinks, t, a, e, y):
            sinks[a](b, 2 * e + t, y)

        passes = []
        for u in items:
            sinks = (P(put_q, u), P(put_v, u)) if u < 4 else (P(put_k, 2 * u - 8), P(put_k, 2 * u - 7))
            for t in range(2):
                passes += quad(wq_t[u] if u < 4 else wk_t, xn_s[b % 2], (u == 5) * GR, GR, tiles[t],
                               P(done, sinks, t))
        return rounds(passes)

    def ln1(b):
        return ln_stats(x_v[b], st_s[b % 2]) + ln_operands(x_v[b], st_s[b % 2], xn_s[b % 2])

    def key_splats(h, odd):
        def job(d):
            for t in range(NV // 128):
                row = kf_s[z, h, t, pl.ds(4 * odd + d, 1), :]
                kb_s[odd][0, d, pl.ds(16 * t, 16)] = jnp.broadcast_to(row, (128, 128)).T.reshape(16, 8, 128)
        return [P(job, d) for d in range(DH)]

    def vpu_scores(h, b, odd, keys, step, nq):
        def job(cs, r):
            n = min(step, keys - r)
            acc = {c: sh_s[b][pl.ds(z, 1), h, :, tiles[c]] for c in cs}
            for d in range(DH):
                k = kb_s[odd][z, d, pl.ds(r // 8, n // 8)]
                for c in cs:
                    q = qf_s[b][z, h, pl.ds(4 * odd + d, 1), tiles[c]]
                    acc[c] = acc[c] + k * lax.broadcast_in_dim(q, k.shape, (1, 2))
            for c in cs:
                p = jnp.exp2(acc[c]).reshape(n, 128)
                p_s[b][pl.ds(odd * S + r, n), tiles[c]] = p
                k_s[0, _at(32 * z + c % nq * n, n), :] = pltpu.bitcast(p, U32)
        nc, nr = NT // nq, -(-keys // step)
        return [P(job, range(n % nc * nq, (n % nc + 1) * nq), (n // nc + nr // nc * (n % nc)) % nr * step)
                for n in range(nc * nr)]

    def mxu_scores(h, b, odd, spans):
        for span in spans:
            ks = []
            for i in span:
                if ks:
                    yield
                ks.append(k_s.at[z][_at(PAD + h * (S // 2) + i // 2, 8), 0:32])
            p = jnp.exp2(dot(_unpack(jnp.concatenate(ks, axis=0)), _unpack(q_s[b].at[z][_at(h * 16, 16), :])))
            n = sum(i >= NV for i in span)
            p_s[b][pl.ds(span[0], 16 * n), :] = p[:16 * n]
            if n < len(span):
                p_s[b][pl.ds(odd * S + span[n], 16 * (len(span) - n)), :] = p[16 * n:]
            yield

    def weighted_values(h, b, odd, dst):
        acc = None
        for j in list(range(NV // KT, NJ)) + list(range(NV // KT)):
            p = p_s[b][pl.ds(j * KT + (odd * S if j * KT < NV else 0), KT), :]
            yield
            d = dot(_unpack(v_s.at[z][_at(PAD + (h * NB + j // NT) * 16, 16), tiles[j % NT]]), p)
            acc = d if acc is None else d + acc
            if j == NV // KT - 1:
                dst[...] = acc
            yield

    def attn_unit(h, b, odd, extra):
        keys, step, nq = (208, 24, 1) if b == NB - 1 else (NV, 16, 2)
        spans = [list(range(NV + 112 * j, NV + 112 * (j + 1), 16)) for j in range(NJ)]
        rest = range(keys, NV, 16)
        for n, i in enumerate(rest):
            spans[(2 * n + 1) * NJ // (2 * len(rest))].append(i)
        qk, pv = mxu_scores(h, b, odd, spans), weighted_values(h - 1, b, 1 - odd, o_s.at[h - 1, b])
        side = vpu_scores(h, b, odd, keys, step, nq)
        total, now, sent = 9 * NJ + len(rest), min(len(rest), 1), 0
        for j in range(NJ):
            if extra and j % 2 == 0 and (b, j) != (0, 0):
                extra.pop(0)()
            next(pv)
            for gen, slots in [(qk, 1)] * len(spans[j]) + [(pv, 2)]:
                next(gen)
                now += slots
                while sent < len(side) and (sent + 1) * total <= now * len(side):
                    side[sent]()
                    sent += 1

    def head_step(h, carry):
        for odd in (0, 1):
            @pl.when(h % 2 == odd)
            def _():
                extra = key_splats(jnp.minimum(h + 1, H - 1), 1 - odd)
                for b in range(NB):
                    attn_unit(h, b, odd, extra)
        return carry

    def exact_unit(u, carry):
        h, b, c = u // NJ, u // NT % NB, pl.ds(pl.multiple_of(u % NT * 128, 128), 128)
        k = jnp.concatenate([_unpack(kt_s[0].at[0][_at(h * 16, 16), 0:128]).T,
                             _unpack(k_s.at[0][_at(PAD + h * (S // 2) + 64, S // 2 - 64), 0:32])], axis=0)
        v = jnp.concatenate([v_s.at[0][_at(PAD + (h * NB + i) * 16, 16), :] for i in range(NB)], axis=1)
        q = qf_s[0][0, h, :, c]
        for i in range(1, NB):
            q = jnp.where(b == i, qf_s[i][0, h, :, c], q)
        s = _matmul(k, q.astype(BF16))
        p = jnp.exp2(s - jnp.max(s, axis=0, keepdims=True))
        o_s[h, b, :, c] = _matmul(_unpack(v), p.astype(BF16))
        return carry

    def normalize(b, safe, pin):
        def job(p):
            for c in tiles:
                ev, od = o_s[2 * p, b, :, c], o_s[2 * p + 1, b, :, c]
                if p == H // 2 - 1:
                    od = jnp.where(safe, ol_s[b][z, :, c], od)
                inv = 1.0 / jnp.where(_low(od[:8]), od[:8], ev[24:])
                ev, od = ev * inv[7:8], od * inv[0:1]
                on_s[0, pl.ds(2 * DH * p, 2 * DH), c] = jnp.concatenate(
                    [ev[:24], jnp.where(_low(inv), ev[24:], od[:8]), od[8:]], axis=0)
        return window([P(job, p) for p in range(H // 2)], o_s.at[H + z, 0], (on_s, 0), pin)

    def wo_mix(wa, wb):
        (ta, a1, a2, ua, va), (tb, b1, b2, ub, vb) = wa, wb
        ta, ua, va, tb, ub, vb = (w.astype(F32) for w in (ta, ua, va, tb, ub, vb))
        left = lax.broadcasted_iota(jnp.int32, ta.shape, 1) < 64
        return (jnp.where(left, tb, ta), a1, a2, jnp.where(left, ua, ua - ub), b1, b2, jnp.where(left, vb, vb - va))

    def out_project(b):
        def steps(u, c, acc):
            def mm(*spans):
                return dot(lhs_queue.pop(), jnp.concatenate([on_s[z, lo:hi, c] for lo, hi in spans], axis=0))

            shared = mm((320, 448))
            for a in range(2):
                y = shared
                for spans in (((0, 128),), ((128, 256),), ((256, 320), (320 + 64 * a, 384 + 64 * a))):
                    yield
                    y = mm(*spans) + y
                rows = pl.ds((2 * u + a) * GR, GR)
                y = y + x_v[b].at[0][rows, c].astype(F32)
                h_s[b % 2][0, rows, c] = y
                ln_add(acc, st_s[0], c, y)
            yield

        gens = [(u, steps(u, c, acc)) for c, acc in [(c, {}) for c in tiles] for u in range(2)]
        return rounds([(wo_t, u * GR, GR, t, gen) for u, gen in gens for t in range(7)])

    def ln2(b, pin):
        return window(ln_operands(h_s[b % 2], st_s[0], xn_s[1]), spare(h_s[b % 2]), (xn_s[1], 0), pin)

    def prep_bias(src, dst, c0, n):
        dst[0, pl.ds(PAD + c0, n), :] = jnp.broadcast_to(src[...].astype(F32)[None, c0:c0 + n], (128, n)).T

    def prep_w2(r, c):
        n = min(256, F // 2 - c)
        (a11, a12), (a21, a22) = ([w2t_v[pl.ds(r0, 16), pl.ds(c0, n)].astype(F32) for c0 in (c, F // 2 + c)]
                                  for r0 in (r, D // 2 + r))
        for i, a in enumerate((a11 + a22, a21 + a22, a11, a22, a11 + a12, a21 - a11, a12 - a22)):
            w2_t.at[0][pl.ds(PAD + (i * (D // 2) + r) // 2, 8), pl.ds(c, n)] = _pack(a)

    def mlp_up():
        def done(r, t, act, a, e, u):
            u = jnp.maximum(u, 0.0)
            act.append(u * u)
            b12, b11, b21, b22 = act + [None] * (4 - len(act))
            new = ({} if b11 is None else {1: b11, 5: b11 - b12} if b21 is None else {3: b21 - b11} if b22 is None
                   else {0: b11 - b22, 2: b22 - b12, 4: b22, 6: b21 - b22})
            for n, v in new.items():
                a_s[t].at[0][pl.ds(r // 2, 32), n * 128:(n + 1) * 128] = _pack(v)

        return rounds([entry for t in range(2) for r in range(0, F // 2, 64)
                       for entry in quad(w1_t, xn_s[1], r, 64, tiles[t], P(done, r, t, []), b1_c)])

    stores = []

    def mlp_down(b):
        def steps(r, t):
            def prod(n, acc=None):
                for k in range(7):
                    if (n, k) != (1, 0):
                        yield
                    y = dot(lhs_queue.pop(), _unpack(a_s[t].at[z][pl.ds(64 * k, 64), n * 128:(n + 1) * 128]))
                    acc = y if acc is None else y + acc
                return acc

            def emit(e, r0, y):
                rows, c = pl.ds(r0, GR), tiles[2 * e + t]
                out_v[b, rows, c] = (y + h_s[b % 2][4 * z, rows, c] + b2_c[z, pl.ds(PAD + r0, GR), :]).astype(BF16)
                if t == 1:
                    stores.append(pltpu.make_async_copy(
                        out_v.at[b, rows, pl.ds(e * HB, HB)], out_hbm.at[rows, pl.ds(b * TB + e * HB, HB)], out_sem))
                    stores[-1].start()

            m2 = yield from prod(1)
            m4 = yield from prod(3)
            emit(0, D // 2 + r, m2 + m4)
            m1 = yield from prod(0)
            c11, c22 = m4 + m1, m1 - m2
            c11 = yield from prod(6, c11)
            m5 = yield from prod(4)
            emit(0, r, c11 + m5)
            m3 = yield from prod(2)
            emit(1, r, m5 - m3)
            c22 = yield from prod(5, c22 + m3)
            emit(1, D // 2 + r, -c22)
            yield

        gens = [(r, steps(r, t)) for t in range(2) for r in range(0, D // 2, GR)]
        return rounds([(w2_t, n * (D // 2) + r, GR, k, gen)
                       for r, gen in gens for n in (1, 3, 0, 6, 4, 2, 5) for k in range(7)])

    mm = project(0, range(6))
    arrive(0)
    _run(ln1(0))
    arrive(1)
    _run([P(prep_qv, 0), P(prep_qv, 128)] + mm[:63])
    arrive(2)
    _run([P(prep_qv, 256), P(prep_qv, 384)] + mm[63:133])
    arrive(3)
    for c in range(384, 2 * D, 128):
        prep_raw(wqkv_v, wk_raw, c, 128, c - 384)
    side = ln1(1)
    _run(mm[133:182], window(side[:16], spare(x_v[1]), None, wq_t[3], 8),
         (mix_raw(w_mix, wk_raw, wk_t, 64, wq_t[3]), 0.7, 1.0))
    _run(mm[182:], window(side[16:], spare(x_v[1]), (xn_s[1], 0), wk_t, 8))
    mm = project(1, range(6))
    _run(mm[:63])
    arrive(4)
    for c in range(0, D, 128):
        prep_raw(wo_v, wo_raw, c, min(128, D - c), c)
    for c in range(0, F, 256):
        prep_bias(b1_v, b1_c, c, 256)
    prep_bias(b2_v, b2_c, 0, D)
    for b, jobs in ((2, mm[63:]), (3, project(2, range(6)))):
        _run(jobs, (window(ln1(b), spare(x_v[b]), (xn_s[b % 2], 0), None, 6), 0.05, 0.97))
    _run(project(3, (4, 5, 0, 1, 2, 3)), (mix_raw(wo_mix, wo_raw, wo_t, 0, None), 0.1, 1.0))
    _run([P(keys_to_rows, h, b) for b in range(NB) for h in range(H)] + key_splats(0, 0))
    o_s[H - 1] = jnp.zeros(o_s.shape[1:], F32)
    arrive(5)

    spans = [range(i, i + 128, 16) for i in range(NV, S - 128, 128)]
    spans.append(list(range(S - 128, S, 16)) + list(range(192, NV, 16)))
    for b in range(NB):
        _run([P(next, mxu_scores(0, b, 0, spans))] * ((S - 192) // 16),
             (vpu_scores(0, b, 0, 192, 16, 2), 0.016, 1.016))
    _run(key_splats(1, 1))
    safe = jnp.max(unsafe[0]) < 0.5
    lax.fori_loop(1, jnp.where(safe, H, 1), head_step, 0)
    lax.fori_loop(0, jnp.where(safe, 0, H * NJ), exact_unit, 0)
    recent.clear()

    pv = [P(_run, [P(next, gen)] * 2) for gen in [weighted_values(H - 1, b, 1, ol_s[b].at[0]) for b in range(NB)]
          for _ in range(NJ)]
    for c in range(0, F // 2, 128):
        prep_quad(w1_v, c, F // 2 + c, 128, [(w1_t, c, 0, 128)])
    side = normalize(0, safe, v_s)
    _run(pv[:20], side[:7])
    _run(side[7:8] + pv[20:23])
    _run(out_project(0))
    _run(pv[23:39], (ln2(0, v_s), 0.3, 1.0))
    for b in range(NB):
        side = [normalize(b + 1, safe, b1_c)] if b + 1 < NB else []
        if b == 0:
            jobs = [P(prep_w2, r, c) for r in range(0, D // 2, 16) for c in range(0, F // 2, 256)]
            side.append((window(jobs, w2t_v.at[_at(64 * z + D, 16)], (w2_t, PAD), b1_c), 0.0, 0.97))
        _run(mlp_up(), *side)
        if b + 1 < NB:
            _run(out_project(b + 1))
            _run(mlp_down(b), (ln2(b + 1, b2_c), 0.1, 0.97), [] if b else pv[39:])
        else:
            _run(mlp_down(b))
    for cp in stores:
        cp.wait()


@jax.jit
def pallas_sequential_preLN__softmax_full_mha__dense_activation_squared_relu__prompt_kernel(
    A_x: jax.Array,
    A_wqkv: jax.Array,
    A_wo: jax.Array,
    B_x: jax.Array,
    B_w1: jax.Array,
    B_b1: jax.Array,
    B_w2: jax.Array,
    B_b2: jax.Array,
):
    del B_x
    hbm = pl.BlockSpec(memory_space=pltpu.HBM)
    vmem = pltpu.VMEM
    out_t = pl.pallas_call(
        _kernel,
        out_shape=jax.ShapeDtypeStruct((D, S), BF16),
        in_specs=[hbm] * 7,
        out_specs=hbm,
        scratch_shapes=[
            [vmem((1, D + 16, TB), BF16)] * NB,
            vmem((D, 3 * D), BF16),
            vmem((D, D), BF16),
            vmem((D, F), BF16),
            vmem((D + 32, F), BF16),
            [vmem((1, PAD + 64, 13 * 128), U32)] * 4,
            vmem((1, PAD + 256, 5 * 128), U32),
            vmem((1, PAD + 128, 13 * 128), U32),
            vmem((1, PAD + D // 2, 5 * 128), U32),
            vmem((1, PAD + 128, 7 * 128), U32),
            vmem((1, PAD + F // 4, 13 * 128), U32),
            vmem((1, PAD + 800, F // 2), U32),
            vmem((1, PAD + F, 128), F32),
            vmem((1, PAD + D, 128), F32),
            [vmem((1, 640, HB), U32)] * 2,
            [vmem((1, 16, TB), F32)] * 2,
            [vmem((1, H * 16, TB), U32)] * NB,
            [vmem((1, H, 32, TB), F32)] * NB,
            [vmem((1, H, 8, TB), F32)] * NB,
            [vmem((1, H * 16, TB), U32)] * NB,
            vmem((1, PAD + H * S // 2, 128), U32),
            vmem((1, H, NV // 128, 32, 128), F32),
            [vmem((1, DH, NV // 8, 8, 128), F32)] * 2,
            vmem((1, PAD + H * NB * 16, TB), U32),
            [vmem((S + NV, TB), F32)] * NB,
            vmem((H + 1, NB, 32, TB), F32),
            [vmem((1, 32, TB), F32)] * NB,
            vmem((1, D, TB), F32),
            [vmem((1, D + 16, TB), F32)] * 2,
            [vmem((1, F // 4, 7 * 128), U32)] * 2,
            vmem((NB, D, TB), BF16),
            vmem((F,), BF16),
            vmem((D,), BF16),
            pltpu.SMEM((2,), jnp.int32),
            pltpu.SemaphoreType.DMA((6,)),
            pltpu.SemaphoreType.DMA(()),
        ],
        compiler_params=pltpu.CompilerParams(vmem_limit_bytes=100 * 1024 * 1024),
        name="fused_block",
    )(A_x.reshape(S, D).T, A_wqkv, A_wo, B_w1, B_b1, B_w2.T, B_b2)
    return out_t.T.reshape(1, S, D)
```

```python
import functools
import math

import jax
import jax.numpy as jnp
from jax import lax
import jax.experimental.pallas as pl
import jax.experimental.pallas.tpu as pltpu

S, D, H, F = 2048, 448, 16, 1792
DH = D // H
TB = 512
HB = TB // 2
NB = S // TB
NT = TB // 128
KT = 128
NJ = S // KT
GH = 4
GR = GH * DH
NV = 256
PAD = 32
EPS = 1e-5
QSCALE = DH ** -0.5 * math.log2(math.e)
BOUND = 40.0
F32, BF16, U32 = jnp.float32, jnp.bfloat16, jnp.uint32
P = functools.partial


def _pack(x):
    return pltpu.bitcast(x.astype(BF16), U32)


def _unpack(w):
    return pltpu.bitcast(w, BF16)


def _round(x):
    return x.astype(BF16).astype(F32)


def _matmul(a, b):
    return lax.dot_general(a, b, (((1,), (0,)), ((), ())), preferred_element_type=F32)


def _low(x):
    return lax.broadcasted_iota(jnp.int32, x.shape, 0) < 4


def _at(row, n):
    return pl.ds(pl.multiple_of(row, 8), n)


def _run(*streams):
    timed = []
    for k, stream in enumerate(streams):
        jobs, start, stop = stream if isinstance(stream, tuple) else (stream, 0.0, 1.0)
        timed += [(start + (stop - start) * (n + 0.5) / len(jobs), k, n, job) for n, job in enumerate(jobs)]
    for entry in sorted(timed, key=lambda e: e[:3]):
        entry[3]()


def _kernel(x_hbm, wqkv_hbm, wo_hbm, w1_hbm, b1_hbm, w2t_hbm, b2_hbm, out_hbm,
            x_v, wqkv_v, wo_v, w1_v, w2t_v, wq_t, wk_raw, wk_t, wo_raw, wo_t, w1_t, w2_t, b1_c, b2_c,
            xn_s, st_s, q_s, qf_s, sh_s, kt_s, k_s, kf_s, kb_s, v_s, p_s, o_s, ol_s, on_s, h_s, a_s, out_v,
            b1_v, b2_v, z_s, in_sem, out_sem):
    def x_copy(b):
        return x_hbm.at[:, b * TB:(b + 1) * TB], x_v[b].at[0, 0:D]

    def w_copy(lo, hi):
        return wqkv_hbm.at[:, lo:hi], wqkv_v.at[:, lo:hi]

    loads = [[pltpu.make_async_copy(src, dst, in_sem.at[n]) for src, dst in group] for n, group in enumerate((
        (x_copy(0),),
        (w_copy(0, 256), w_copy(896, 1152)),
        (w_copy(256, 512), w_copy(1152, None)),
        (w_copy(512, 896), x_copy(1)),
        (x_copy(2), x_copy(3), (wo_hbm, wo_v), (b1_hbm, b1_v), (b2_hbm, b2_v)),
        ((w1_hbm, w1_v), (w2t_hbm, w2t_v.at[0:D]))))]
    for group in loads:
        for cp in group:
            cp.start()

    def arrive(n):
        for cp in loads[n]:
            cp.wait()

    def set_zero(i, carry):
        z_s[i] = 0
        return carry

    lax.fori_loop(0, 2, set_zero, 0)
    z = z_s[0]
    tiles = [slice(c, c + 128) for c in range(0, TB, 128)]
    recent = []
    streaming = [None]
    lhs_queue = []

    def dot(a, b):
        y = _matmul(a, b)
        recent.extend((y, c) for c in tiles[:y.shape[1] // 128])
        return y

    def window(jobs, src, dst, pin, back=20):
        out = [None]

        def step(n):
            if n > 0:
                ref = streaming[0] if pin is None else pin
                w = dst[0][0, _at(32 * z + dst[1], 8), 0:128] if out[0] is None else out[0]
                ref[0, _at(64 * z, 8), 0:w.shape[1]] = w if w.dtype == ref.dtype else pltpu.bitcast(w, ref.dtype)
            if n < len(jobs):
                if len(recent) >= back:
                    y, c = recent[-back]
                    w = y[-8:, c] if src.dtype == F32 else pltpu.bitcast(y[-8:, c], src.dtype)
                    src[pl.ds(0, w.shape[0]), 0:128] = w
                out[0] = jobs[n]()
        return [P(step, n) for n in range(len(jobs) + 1)]

    def spare(ref):
        return ref.at[5 * z, pl.ds(D, 16)]

    def stream(passes):
        def job(w, r0, n, c, consumer):
            lhs_queue.append(_unpack(w.at[z][pl.ds(PAD + r0 // 2, n // 2), c * 128:(c + 1) * 128]))
            next(consumer)
        return [P(job, *entry) for entry in passes]

    def fine_stream(passes):
        def job(group, got, i):
            streaming[0] = group[-1][0]
            for (w, r0, _, c, _), rows in zip(group, got):
                rows.append(w.at[z][pl.ds(PAD + r0 // 2 + 8 * i, 8), c * 128:(c + 1) * 128])
            if 16 * (i + 1) == group[0][2]:
                for entry, rows in zip(group, got):
                    lhs_queue.append(_unpack(jnp.concatenate(rows, axis=0)))
                    next(entry[4])
        jobs = []
        for k in range(0, len(passes), 4):
            got = [[] for _ in range(4)]
            jobs += [P(job, passes[k:k + 4], got, i) for i in range(passes[k][2] // 16)]
        return jobs

    def ln_add(acc, st, c, x):
        if not acc:
            acc.update(c=x[0:1], n=0)
        d = x - acc["c"]
        for key, v in (("s1", d), ("s2", d * d)):
            v = jnp.sum(v.reshape(-1, 8, x.shape[1]), axis=0)
            acc[key] = v if acc["n"] == 0 else acc[key] + v
        acc["n"] += x.shape[0]
        if acc["n"] == D:
            m = jnp.sum(acc["s1"], axis=0, keepdims=True) * (1.0 / D)
            var = jnp.sum(acc["s2"], axis=0, keepdims=True) * (1.0 / D) - m * m
            st[0, 0:8, c] = jnp.broadcast_to(m + acc["c"], acc["s1"].shape)
            st[0, 8:16, c] = jnp.broadcast_to(lax.rsqrt(jnp.maximum(var, 0.0) + EPS), acc["s1"].shape)
        return acc["s2"]

    def ln_stats(src, st):
        def job(acc, c, r):
            return ln_add(acc, st, c, src.at[z][r:r + 32, c].astype(F32))
        return [P(job, acc, c, r) for acc, c in (({}, slice(0, HB)), ({}, slice(HB, TB))) for r in range(0, D, 32)]

    def ln_operands(src, st, dst):
        def rows(e, r0, n):
            c = slice(e * HB, (e + 1) * HB)
            x = src.at[3 * z][r0:r0 + n, c].astype(F32).reshape(n // 8, 8, HB)
            return ((x - st[z, 0:8, c][None]) * st[z, 8:16, c][None]).reshape(n, HB)

        def put(t, r, val):
            dst.at[0][pl.ds(64 * t + r // 2, val.shape[0] // 2), :] = _pack(val)

        def mixed(r):
            (x1, x2), (y1, y2) = ([rows(e, o + r, 16) for o in (0, 128)] for e in range(2))
            for t, v in zip((0, 1, 2, 4, 5, 6, 7), (y2, y1 - y2, x2 + y2, x1 + y2, x2 - x1, x1, x1 + y1)):
                put(t, r, v)

        def own(e):
            put((3, 8)[e], 0, rows(e, 256, 64))

        def shared(r):
            e = (r - 320) // 64
            other = _round(rows(1 - e, r, 32))
            put(9, r - 320, other)
            put((3, 8)[e], 64 + r % 64, rows(e, r, 32) - other)

        return ([P(mixed, r) for r in range(0, 128, 16)] + [P(own, 0), P(own, 1)]
                + [P(shared, r) for r in range(320, D, 32)])

    def w_tiles(src, c):
        return (src[320:448, c], src[0:128, c], src[128:256, c], src[256:384, c],
                jnp.concatenate([src[256:320, c], src[384:448, c]], axis=0))

    def w_mix(wa, wb):
        (ta, a11, a12, ua, va), (tb, a21, a22, ub, vb) = wa, wb
        f11, f12, f21, f22 = (w.astype(F32) for w in (a11, a12, a21, a22))
        return (ta, va, f11 + f12, a11, f12 - f22, ua, f11 + f22, a22, f21 + f22, tb, ub, f21 - f11, vb)

    def prep_quad(src, ca, cb, n, dsts):
        for t, w in enumerate(w_mix(w_tiles(src, slice(ca, ca + n)), w_tiles(src, slice(cb, cb + n)))):
            w = pltpu.bitcast(w.astype(BF16).T, U32)
            for dst, r0, lo, hi in dsts:
                dst.at[0][pl.ds(PAD + r0 // 2, (hi - lo) // 2), t * 128:(t + 1) * 128] = w[lo // 2:hi // 2]

    def prep_raw(src, dst, c0, n, r0):
        for t, w in enumerate(w_tiles(src, slice(c0, c0 + n))):
            dst.at[0][pl.ds(PAD + r0 // 2, n // 2), t * 128:(t + 1) * 128] = pltpu.bitcast(w.T, U32)

    def mix_raw(mix, raw, dst, first, pin):
        def job(r):
            wa, wb = ([_unpack(raw.at[z][pl.ds(PAD + (first + r // GR * GR + r + o) // 2, 8), c:c + 128])
                       for c in range(0, 640, 128)] for o in (0, GR))
            for t, w in enumerate(mix(wa, wb)):
                dst.at[0][pl.ds(PAD + r // 2, 8), t * 128:(t + 1) * 128] = _pack(w)
        return window([P(job, r) for r in range(0, 2 * GR, 16)], raw.at[5 * z], (dst, PAD), pin, 8)

    def quad(w, src, r0, n, cols, done, bias=None):
        gen = mm_quad(src, r0, n, cols, done, bias)
        return [(w, r0, n, c, gen) for c in range(13)]

    def mm_quad(src, r0, n, cols, done, bias):
        def mm(t):
            return dot(lhs_queue.pop(), _unpack(src.at[z][pl.ds(64 * t, 64), cols]))

        ta = mm(9)
        if bias is not None:
            ta = ta + bias[z, pl.ds(r0 + PAD, n), :]
        yield
        ay = mm(8) + ta
        yield
        m5 = mm(0)
        ax, ay = ta - m5, ay + m5
        yield
        m3 = mm(1)
        done(0, 1, ay + m3)
        yield
        ax = mm(2) + ax
        yield
        ax = mm(3) + ax
        yield
        m1 = mm(4)
        ax, by = ax + m1, m3 + m1
        yield
        m4 = mm(5)
        done(0, 0, ax + m4)
        yield
        m2 = mm(6)
        bx, by = m4 + m2, by - m2
        yield
        tb = mm(9)
        if bias is not None:
            tb = tb + bias[z, pl.ds(F // 2 + r0 + PAD, n), :]
        bx, by = bx + tb, by + tb
        yield
        done(1, 0, mm(3) + bx)
        yield
        by = mm(7) + by
        yield
        done(1, 1, mm(8) + by)
        yield

    unsafe = [jnp.zeros((8, 128), F32)]

    def split_pair(y, p, fill):
        r = 2 * DH * p
        mid = y[r + 24:r + 32]
        return (jnp.concatenate([y[r:r + 24], jnp.where(_low(mid), mid, fill)], axis=0),
                jnp.concatenate([jnp.where(_low(mid), fill, mid), y[r + 32:r + 56]], axis=0))

    def checked_norm(w, scale):
        n2 = jnp.broadcast_to(jnp.sum(w * w, axis=0, keepdims=True), (8, 128)) * scale
        unsafe[0] = jnp.where(n2 <= BOUND, unsafe[0], 1.0)
        return n2

    def put_q(g, b, t, q):
        q = q * QSCALE
        for p in range(2):
            for e, w in enumerate(split_pair(q, p, 0.0)):
                h = g * GH + 2 * p + e
                shift = _round((checked_norm(w, 1.0 / QSCALE) + BOUND) * -0.5)
                qf_s[b][0, h, :, tiles[t]] = w
                sh_s[b][0, h, :, tiles[t]] = shift
                q_s[b].at[0][pl.ds(h * 16, 16), tiles[t]] = _pack(split_pair(q, p, 0.25 * shift)[e])

    def put_k(g, b, t, k):
        for p in range(2):
            for e, w in enumerate(split_pair(k, p, 0.0)):
                h = g * GH + 2 * p + e
                checked_norm(w, QSCALE)
                kt_s[b].at[0][pl.ds(h * 16, 16), tiles[t]] = _pack(split_pair(k, p, 1.0)[e])
                if b * TB + t * 128 < NV:
                    kf_s[0, h, t] = w

    def put_v(g, b, t, v):
        for p in range(2):
            for e, w in enumerate(split_pair(v, p, 1.0)):
                v_s.at[0][pl.ds(PAD + ((g * GH + 2 * p + e) * NB + b) * 16, 16), tiles[t]] = _pack(w)

    def keys_to_rows(h, b):
        lo = 128 if b == 0 else 0
        k = pltpu.bitcast(_unpack(kt_s[b].at[z][pl.ds(h * 16, 16), lo:]).T, U32)
        k_s.at[0][pl.ds(PAD + (h * S + b * TB + lo) // 2, (TB - lo) // 2), 0:32] = k

    def prep_qv(c):
        n = min(128, D - c)
        prep_quad(wqkv_v, c, 2 * D + c, n,
                  [(wq_t[g], max(c - g * GR, 0), max(g * GR - c, 0), min((g + 1) * GR - c, n))
                   for g in range(c // GR, (c + n - 1) // GR + 1)])

    def project(b, items):
        def done(sinks, t, a, e, y):
            sinks[a](b, 2 * e + t, y)

        passes = []
        for u in items:
            sinks = (P(put_q, u), P(put_v, u)) if u < 4 else (P(put_k, 2 * u - 8), P(put_k, 2 * u - 7))
            for t in range(2):
                passes += quad(wq_t[u] if u < 4 else wk_t, xn_s[b % 2], (u == 5) * GR, GR, tiles[t],
                               P(done, sinks, t))
        return fine_stream(passes)

    def ln1(b):
        return ln_stats(x_v[b], st_s[b % 2]) + ln_operands(x_v[b], st_s[b % 2], xn_s[b % 2])

    def key_splats(h, odd):
        def job(d):
            for t in range(NV // 128):
                row = kf_s[z, h, t, pl.ds(4 * odd + d, 1), :]
                kb_s[odd][0, d, pl.ds(16 * t, 16)] = jnp.broadcast_to(row, (128, 128)).T.reshape(16, 8, 128)
        return [P(job, d) for d in range(DH)]

    def vpu_scores(h, b, odd, keys, step, nq):
        def job(cs, r):
            n = min(step, keys - r)
            acc = {c: sh_s[b][pl.ds(z, 1), h, :, tiles[c]] for c in cs}
            for d in range(DH):
                k = kb_s[odd][z, d, pl.ds(r // 8, n // 8)]
                for c in cs:
                    q = qf_s[b][z, h, pl.ds(4 * odd + d, 1), tiles[c]]
                    acc[c] = acc[c] + k * lax.broadcast_in_dim(q, k.shape, (1, 2))
            for c in cs:
                p = jnp.exp2(acc[c]).reshape(n, 128)
                p_s[b][pl.ds(odd * S + r, n), tiles[c]] = p
                k_s[0, _at(32 * z + c % nq * n, n), :] = pltpu.bitcast(p, U32)
        nc, nr = NT // nq, -(-keys // step)
        return [P(job, range(n % nc * nq, (n % nc + 1) * nq), (n // nc + nr // nc * (n % nc)) % nr * step)
                for n in range(nc * nr)]

    def mxu_scores(h, b, odd, spans):
        for span in spans:
            ks = []
            for i in span:
                if ks:
                    yield
                ks.append(k_s.at[z][_at(PAD + h * (S // 2) + i // 2, 8), 0:32])
            p = jnp.exp2(dot(_unpack(jnp.concatenate(ks, axis=0)), _unpack(q_s[b].at[z][_at(h * 16, 16), :])))
            n = sum(i >= NV for i in span)
            p_s[b][pl.ds(span[0], 16 * n), :] = p[:16 * n]
            if n < len(span):
                p_s[b][pl.ds(odd * S + span[n], 16 * (len(span) - n)), :] = p[16 * n:]
            yield

    def weighted_values(h, b, odd, dst):
        acc = None
        for j in list(range(NV // KT, NJ)) + list(range(NV // KT)):
            p = p_s[b][pl.ds(j * KT + (odd * S if j * KT < NV else 0), KT), :]
            yield
            d = dot(_unpack(v_s.at[z][_at(PAD + (h * NB + j // NT) * 16, 16), tiles[j % NT]]), p)
            acc = d if acc is None else d + acc
            if j == NV // KT - 1:
                dst[...] = acc
            yield

    def attn_unit(h, b, odd, extra):
        keys, step, nq = (208, 24, 1) if b == NB - 1 else (NV, 16, 2)
        spans = [list(range(NV + 112 * j, NV + 112 * (j + 1), 16)) for j in range(NJ)]
        rest = range(keys, NV, 16)
        for n, i in enumerate(rest):
            spans[(2 * n + 1) * NJ // (2 * len(rest))].append(i)
        qk, pv = mxu_scores(h, b, odd, spans), weighted_values(h - 1, b, 1 - odd, o_s.at[h - 1, b])
        side = vpu_scores(h, b, odd, keys, step, nq)
        total, now, sent = 9 * NJ + len(rest), 0, 0
        for j in range(NJ):
            if extra and j % 2 == 0 and (b, j) != (0, 0):
                extra.pop(0)()
            next(pv)
            for gen, slots in [(qk, 1)] * len(spans[j]) + [(pv, 2)]:
                next(gen)
                now += slots
                while sent < len(side) and (sent + 1) * total <= now * len(side):
                    side[sent]()
                    sent += 1

    def head_step(h, carry):
        for odd in (0, 1):
            @pl.when(h % 2 == odd)
            def _():
                extra = key_splats(jnp.minimum(h + 1, H - 1), 1 - odd)
                for b in range(NB):
                    attn_unit(h, b, odd, extra)
        return carry

    def exact_unit(u, carry):
        h, b, c = u // NJ, u // NT % NB, pl.ds(pl.multiple_of(u % NT * 128, 128), 128)
        k = jnp.concatenate([_unpack(kt_s[0].at[0][_at(h * 16, 16), 0:128]).T,
                             _unpack(k_s.at[0][_at(PAD + h * (S // 2) + 64, S // 2 - 64), 0:32])], axis=0)
        v = jnp.concatenate([v_s.at[0][_at(PAD + (h * NB + i) * 16, 16), :] for i in range(NB)], axis=1)
        q = qf_s[0][0, h, :, c]
        for i in range(1, NB):
            q = jnp.where(b == i, qf_s[i][0, h, :, c], q)
        s = _matmul(k, q.astype(BF16))
        p = jnp.exp2(s - jnp.max(s, axis=0, keepdims=True))
        o_s[h, b, :, c] = _matmul(_unpack(v), p.astype(BF16))
        return carry

    def normalize(b, safe, pin):
        def job(p):
            for c in tiles:
                ev, od = o_s[2 * p, b, :, c], o_s[2 * p + 1, b, :, c]
                if p == H // 2 - 1:
                    od = jnp.where(safe, ol_s[b][z, :, c], od)
                inv = 1.0 / jnp.where(_low(od[:8]), od[:8], ev[24:])
                ev, od = ev * inv[7:8], od * inv[0:1]
                on_s[0, pl.ds(2 * DH * p, 2 * DH), c] = jnp.concatenate(
                    [ev[:24], jnp.where(_low(inv), ev[24:], od[:8]), od[8:]], axis=0)
        return window([P(job, p) for p in range(H // 2)], o_s.at[H + z, 0], (on_s, 0), pin)

    def wo_mix(wa, wb):
        (ta, a1, a2, ua, va), (tb, b1, b2, ub, vb) = wa, wb
        ta, ua, va, tb, ub, vb = (w.astype(F32) for w in (ta, ua, va, tb, ub, vb))
        left = lax.broadcasted_iota(jnp.int32, ta.shape, 1) < 64
        return (jnp.where(left, tb, ta), a1, a2, jnp.where(left, ua, ua - ub), b1, b2, jnp.where(left, vb, vb - va))

    def out_project(b):
        def steps(u, c, acc):
            def mm(*spans):
                return dot(lhs_queue.pop(), jnp.concatenate([on_s[z, lo:hi, c] for lo, hi in spans], axis=0))

            shared = mm((320, 448))
            for a in range(2):
                y = shared
                for spans in (((0, 128),), ((128, 256),), ((256, 320), (320 + 64 * a, 384 + 64 * a))):
                    yield
                    y = mm(*spans) + y
                rows = pl.ds((2 * u + a) * GR, GR)
                y = y + x_v[b].at[0][rows, c].astype(F32)
                h_s[b % 2][0, rows, c] = y
                ln_add(acc, st_s[0], c, y)
            yield

        gens = [(u, steps(u, c, acc)) for c, acc in [(c, {}) for c in tiles] for u in range(2)]
        return stream([(wo_t, u * GR, GR, t, gen) for u, gen in gens for t in range(7)])

    def ln2(b, pin):
        return window(ln_operands(h_s[b % 2], st_s[0], xn_s[1]), spare(h_s[b % 2]), (xn_s[1], 0), pin)

    def prep_bias(src, dst, c0, n):
        dst[0, pl.ds(PAD + c0, n), :] = jnp.broadcast_to(src[...].astype(F32)[None, c0:c0 + n], (128, n)).T

    def prep_w2(r, c):
        n = min(256, F // 2 - c)
        (a11, a12), (a21, a22) = ([w2t_v[pl.ds(r0, 16), pl.ds(c0, n)].astype(F32) for c0 in (c, F // 2 + c)]
                                  for r0 in (r, D // 2 + r))
        for i, a in enumerate((a11 + a22, a21 + a22, a11, a22, a11 + a12, a21 - a11, a12 - a22)):
            w2_t.at[0][pl.ds(PAD + (i * (D // 2) + r) // 2, 8), pl.ds(c, n)] = _pack(a)

    def mlp_up():
        def done(r, t, act, a, e, u):
            u = jnp.maximum(u, 0.0)
            act.append(u * u)
            b12, b11, b21, b22 = act + [None] * (4 - len(act))
            new = ({} if b11 is None else {1: b11, 5: b11 - b12} if b21 is None else {3: b21 - b11} if b22 is None
                   else {0: b11 - b22, 2: b22 - b12, 4: b22, 6: b21 - b22})
            for n, v in new.items():
                a_s[t].at[0][pl.ds(r // 2, 32), n * 128:(n + 1) * 128] = _pack(v)

        return stream([entry for t in range(2) for r in range(0, F // 2, 64)
                       for entry in quad(w1_t, xn_s[1], r, 64, tiles[t], P(done, r, t, []), b1_c)])

    stores = []

    def mlp_down(b):
        def steps(r, t):
            def prod(n, acc=None):
                for k in range(7):
                    if (n, k) != (1, 0):
                        yield
                    y = dot(lhs_queue.pop(), _unpack(a_s[t].at[z][pl.ds(64 * k, 64), n * 128:(n + 1) * 128]))
                    acc = y if acc is None else y + acc
                return acc

            def emit(e, r0, y):
                rows, c = pl.ds(r0, GR), tiles[2 * e + t]
                out_v[b, rows, c] = (y + h_s[b % 2][4 * z, rows, c] + b2_c[z, pl.ds(PAD + r0, GR), :]).astype(BF16)
                if t == 1:
                    stores.append(pltpu.make_async_copy(
                        out_v.at[b, rows, pl.ds(e * HB, HB)], out_hbm.at[rows, pl.ds(b * TB + e * HB, HB)], out_sem))
                    stores[-1].start()

            m2 = yield from prod(1)
            m4 = yield from prod(3)
            emit(0, D // 2 + r, m2 + m4)
            m1 = yield from prod(0)
            c11, c22 = m4 + m1, m1 - m2
            c11 = yield from prod(6, c11)
            m5 = yield from prod(4)
            emit(0, r, c11 + m5)
            m3 = yield from prod(2)
            emit(1, r, m5 - m3)
            c22 = yield from prod(5, c22 + m3)
            emit(1, D // 2 + r, -c22)
            yield

        gens = [(r, steps(r, t)) for t in range(2) for r in range(0, D // 2, GR)]
        return stream([(w2_t, n * (D // 2) + r, GR, k, gen)
                       for r, gen in gens for n in (1, 3, 0, 6, 4, 2, 5) for k in range(7)])

    mm = project(0, range(6))
    arrive(0)
    _run(ln1(0))
    arrive(1)
    _run([P(prep_qv, 0), P(prep_qv, 128)] + mm[:63])
    arrive(2)
    _run([P(prep_qv, 256), P(prep_qv, 384)] + mm[63:133])
    arrive(3)
    for c in range(384, 2 * D, 128):
        prep_raw(wqkv_v, wk_raw, c, 128, c - 384)
    side = ln1(1)
    _run(mm[133:182], window(side[:16], spare(x_v[1]), None, wq_t[3], 8),
         (mix_raw(w_mix, wk_raw, wk_t, 64, wq_t[3]), 0.7, 1.0))
    _run(mm[182:], window(side[16:], spare(x_v[1]), (xn_s[1], 0), wk_t, 8))
    mm = project(1, range(6))
    _run(mm[:63])
    arrive(4)
    for c in range(0, D, 128):
        prep_raw(wo_v, wo_raw, c, min(128, D - c), c)
    for c in range(0, F, 256):
        prep_bias(b1_v, b1_c, c, 256)
    prep_bias(b2_v, b2_c, 0, D)
    for b, jobs in ((2, mm[63:]), (3, project(2, range(6)))):
        _run(jobs, (window(ln1(b), spare(x_v[b]), (xn_s[b % 2], 0), None, 6), 0.05, 0.97))
    _run(project(3, (4, 5, 0, 1, 2, 3)), (mix_raw(wo_mix, wo_raw, wo_t, 0, None), 0.1, 1.0))
    _run([P(keys_to_rows, h, b) for b in range(NB) for h in range(H)] + key_splats(0, 0))
    o_s[H - 1] = jnp.zeros(o_s.shape[1:], F32)
    arrive(5)

    spans = [range(i, i + 128, 16) for i in range(NV, S - 128, 128)]
    spans.append(list(range(S - 128, S, 16)) + list(range(192, NV, 16)))
    for b in range(NB):
        _run([P(next, mxu_scores(0, b, 0, spans))] * ((S - 192) // 16),
             (vpu_scores(0, b, 0, 192, 16, 2), 0.016, 1.016))
    _run(key_splats(1, 1))
    safe = jnp.max(unsafe[0]) < 0.5
    lax.fori_loop(1, jnp.where(safe, H, 1), head_step, 0)
    lax.fori_loop(0, jnp.where(safe, 0, H * NJ), exact_unit, 0)
    recent.clear()

    pv = [P(_run, [P(next, gen)] * 2) for gen in [weighted_values(H - 1, b, 1, ol_s[b].at[0]) for b in range(NB)]
          for _ in range(NJ)]
    for c in range(0, F // 2, 128):
        prep_quad(w1_v, c, F // 2 + c, 128, [(w1_t, c, 0, 128)])
    side = normalize(0, safe, v_s)
    _run(pv[:20], side[:7])
    _run(side[7:8] + pv[20:23])
    _run(out_project(0))
    _run(pv[23:39], (ln2(0, v_s), 0.3, 1.0))
    for b in range(NB):
        side = [normalize(b + 1, safe, b1_c)] if b + 1 < NB else []
        if b == 0:
            jobs = [P(prep_w2, r, c) for r in range(0, D // 2, 16) for c in range(0, F // 2, 256)]
            side.append((window(jobs, w2t_v.at[_at(64 * z + D, 16)], (w2_t, PAD), b1_c), 0.0, 0.97))
        _run(mlp_up(), *side)
        if b + 1 < NB:
            _run(out_project(b + 1))
            _run(mlp_down(b), (ln2(b + 1, b2_c), 0.1, 0.97), [] if b else pv[39:])
        else:
            _run(mlp_down(b))
    for cp in stores:
        cp.wait()


@jax.jit
def pallas_sequential_preLN__softmax_full_mha__dense_activation_squared_relu__prompt_kernel(
    A_x: jax.Array,
    A_wqkv: jax.Array,
    A_wo: jax.Array,
    B_x: jax.Array,
    B_w1: jax.Array,
    B_b1: jax.Array,
    B_w2: jax.Array,
    B_b2: jax.Array,
):
    del B_x
    hbm = pl.BlockSpec(memory_space=pltpu.HBM)
    vmem = pltpu.VMEM
    out_t = pl.pallas_call(
        _kernel,
        out_shape=jax.ShapeDtypeStruct((D, S), BF16),
        in_specs=[hbm] * 7,
        out_specs=hbm,
        scratch_shapes=[
            [vmem((1, D + 16, TB), BF16)] * NB,
            vmem((D, 3 * D), BF16),
            vmem((D, D), BF16),
            vmem((D, F), BF16),
            vmem((D + 32, F), BF16),
            [vmem((1, PAD + 64, 13 * 128), U32)] * 4,
            vmem((1, PAD + 256, 5 * 128), U32),
            vmem((1, PAD + 128, 13 * 128), U32),
            vmem((1, PAD + D // 2, 5 * 128), U32),
            vmem((1, PAD + 128, 7 * 128), U32),
            vmem((1, PAD + F // 4, 13 * 128), U32),
            vmem((1, PAD + 800, F // 2), U32),
            vmem((1, PAD + F, 128), F32),
            vmem((1, PAD + D, 128), F32),
            [vmem((1, 640, HB), U32)] * 2,
            [vmem((1, 16, TB), F32)] * 2,
            [vmem((1, H * 16, TB), U32)] * NB,
            [vmem((1, H, 32, TB), F32)] * NB,
            [vmem((1, H, 8, TB), F32)] * NB,
            [vmem((1, H * 16, TB), U32)] * NB,
            vmem((1, PAD + H * S // 2, 128), U32),
            vmem((1, H, NV // 128, 32, 128), F32),
            [vmem((1, DH, NV // 8, 8, 128), F32)] * 2,
            vmem((1, PAD + H * NB * 16, TB), U32),
            [vmem((S + NV, TB), F32)] * NB,
            vmem((H + 1, NB, 32, TB), F32),
            [vmem((1, 32, TB), F32)] * NB,
            vmem((1, D, TB + 128), F32),
            [vmem((1, D + 16, TB), F32)] * 2,
            [vmem((1, F // 4, 7 * 128), U32)] * 2,
            vmem((NB, D, TB), BF16),
            vmem((F,), BF16),
            vmem((D,), BF16),
            pltpu.SMEM((2,), jnp.int32),
            pltpu.SemaphoreType.DMA((6,)),
            pltpu.SemaphoreType.DMA(()),
        ],
        compiler_params=pltpu.CompilerParams(vmem_limit_bytes=100 * 1024 * 1024),
        name="fused_block",
    )(A_x.reshape(S, D).T, A_wqkv, A_wo, B_w1, B_b1, B_w2.T, B_b2)
    return out_t.T.reshape(1, S, D)
```
